```python
import os as _os
_os.environ.setdefault("JAX_PLATFORMS", "cpu")
import jax
import jax.numpy as jnp

def _softmax(x, axis=-1):
    return jax.nn.softmax(x, axis=axis)
def _gelu(x):
    return jax.nn.gelu(x, approximate=True)
def _silu(x):
    return jax.nn.silu(x)
def _sigmoid(x):
    return jax.nn.sigmoid(x)
def _layernorm(x, axis=-1, eps=1e-5):
    m = jnp.mean(x, axis=axis, keepdims=True)
    v = jnp.var(x, axis=axis, keepdims=True)
    return (x - m) / jnp.sqrt(v + eps)
def _scatter_add(tgt, idx, src, axis=0):
    return tgt.at[idx].add(src)
def _segment_sum(src, seg, n):
    return jax.ops.segment_sum(src, seg, n)
class _Rng:
    def __init__(self, key):
        self._k = key
    def _next(self):
        self._k, sub = jax.random.split(self._k)
        return sub
    def normal(self, shape):
        return jax.random.normal(self._next(), shape, dtype=jnp.bfloat16)
    def randint(self, lo, hi, shape):
        return jax.random.randint(self._next(), shape, lo, hi, dtype=jnp.int32)
    def uniform(self, shape, lo=0.0, hi=1.0):
        return jax.random.uniform(self._next(), shape, jnp.bfloat16, lo, hi)
    def permutation(self, n):
        return jax.random.permutation(self._next(), n)


kernel_name = 'sequential_preLN__softmax_full_mha__glu_gated_swiglu__prompt'

def setup_inputs():
    _rng = _Rng(jax.random.key(int.from_bytes(__import__("os").urandom(4), "little")))
    _w = (lambda a: (lambda t: t.astype(jnp.bfloat16) if jnp.issubdtype(t.dtype, jnp.floating) else t)(jnp.asarray(a)))
    def _A_setup():
        B, S, D = 1, 2048, 640
        return {
            "x": _w((lambda *s: _rng.normal(s) * 0.05)(B, S, D)),
            "wqkv": _w((lambda *s: _rng.normal(s) * 0.05)(D, 3 * D)),
            "wo": _w((lambda *s: _rng.normal(s) * 0.05)(D, D)),
        }
    _A_in = _A_setup()

    def _B_setup():
        B, S, D, F = 1, 2048, 640, 1728
        return {
            "x": _w((lambda *s: _rng.normal(s) * 0.05)(B, S, D)),
            "w1": _w((lambda *s: _rng.normal(s) * 0.05)(D, F) * (2.0 / D) ** 0.5),
            "w3": _w((lambda *s: _rng.normal(s) * 0.05)(D, F) * (2.0 / D) ** 0.5),
            "w2": _w((lambda *s: _rng.normal(s) * 0.05)(F, D) * (2.0 / F) ** 0.5),
        }
    _B_in = _B_setup()

    return {
        "A_x": _A_in["x"],
        "A_wqkv": _A_in["wqkv"],
        "A_wo": _A_in["wo"],
        "B_x": _B_in["x"],
        "B_w1": _B_in["w1"],
        "B_w3": _B_in["w3"],
        "B_w2": _B_in["w2"],
    }

def reference(A_x, A_wqkv, A_wo, B_x, B_w1, B_w3, B_w2):
    def _A_ref(x, wqkv, wo):
        B, S, D = x.shape
        H = 32; Dh = D // H
        qkv = (lambda x, *d: x.transpose(*d))((x @ wqkv).reshape(B, S, 3, H, Dh), 2, 0, 3, 1, 4)
        q, k, v = qkv[0], qkv[1], qkv[2]
        scale = Dh ** -0.5
        scores = jnp.einsum("bhqd,bhkd->bhqk", q, k) * scale
        p = _softmax(scores, axis=-1)
        o = jnp.einsum("bhqk,bhkd->bhqd", p, v)
        return (lambda x, *d: x.transpose(*d))(o, 0, 2, 1, 3).reshape(B, S, D) @ wo

    def _B_ref(x, w1, w3, w2):
        gate = jnp.einsum("bsd,df->bsf", x, w1)
        up = jnp.einsum("bsd,df->bsf", x, w3)
        h = _silu(gate) * up
        out = jnp.einsum("bsf,fd->bsd", h, w2)
        return out

    x = A_x
    h = x + _A_ref(_layernorm(x, axis=-1), A_wqkv, A_wo)
    h2 = h + _B_ref(_layernorm(h, axis=-1), B_w1, B_w3, B_w2)
    return h2
```

```python
import functools
import numpy as np
import jax
import jax.numpy as jnp
from jax import lax
import jax.experimental.pallas as pl
import jax.experimental.pallas.tpu as pltpu

S, D, H, DH, F = 2048, 640, 32, 20, 1728
G = 4
NG = H // G
GW = G * DH
EPS = 1e-5
QSCALE = float(DH ** -0.5 * np.log2(np.e))
BF = jnp.bfloat16
F32 = jnp.float32


def _ln(xf):
    m = jnp.mean(xf, axis=-1, keepdims=True)
    d = xf - m
    v = jnp.mean(d * d, axis=-1, keepdims=True)
    return d * lax.rsqrt(v + EPS)


def _dot(a, b):
    return jnp.dot(a, b, preferred_element_type=F32)


def _dot_nt(a, b):
    return lax.dot_general(a, b, (((1,), (1,)), ((), ())), preferred_element_type=F32)


def make_kernel(TB1=256, BQ=1024, CK=128, HPB=4, TB3=256, FC=256, name="k"):
    NB1 = S // TB1
    NQ = S // BQ
    NB3 = S // TB3
    XCH = 512
    NXC = S // XCH

    def kernel(x_hbm, wqkv_hbm, wo_hbm, w1_hbm, w3_hbm, w2_hbm, out_hbm,
               x_v, wqkv_v, wo_v, w1_v, w3_v, w2_v,
               k_s, qt_s, vt_s, ot_s, out_v, sem_x, sem_w, sem_o):
        def x_cp(i):
            return pltpu.make_async_copy(x_hbm.at[pl.ds(i * XCH, XCH), :], x_v.at[pl.ds(i * XCH, XCH), :], sem_x.at[i])
        def wq_cp(j):
            return pltpu.make_async_copy(wqkv_hbm.at[:, pl.ds(j * D, D)], wqkv_v.at[:, pl.ds(j * D, D)], sem_w.at[j])
        wo_cp = pltpu.make_async_copy(wo_hbm, wo_v, sem_w.at[3])
        w1_cp = pltpu.make_async_copy(w1_hbm, w1_v, sem_w.at[4])
        w3_cp = pltpu.make_async_copy(w3_hbm, w3_v, sem_w.at[5])
        w2_cp = pltpu.make_async_copy(w2_hbm, w2_v, sem_w.at[6])
        x_cp(0).start()
        wq_cp(0).start()
        wq_cp(1).start()
        wq_cp(2).start()
        for i in range(1, NXC):
            x_cp(i).start()
        wo_cp.start(); w1_cp.start(); w3_cp.start(); w2_cp.start()

        qt_s[D:, :] = jnp.zeros((qt_s.shape[0] - D, S), BF)

        x_cp(0).wait()
        wq_cp(0).wait(); wq_cp(1).wait(); wq_cp(2).wait()
        row32 = lax.broadcasted_iota(jnp.int32, (32, TB1), 0)
        for b in range(NB1):
            r0 = b * TB1
            if r0 % XCH == 0 and r0 > 0:
                x_cp(r0 // XCH).wait()
            xh = _ln(x_v[r0:r0 + TB1, :].astype(F32)).astype(BF)
            q = _dot(xh, wqkv_v[:, 0:D]) * QSCALE
            qt_s[0:D, r0:r0 + TB1] = q.astype(BF).T
            k = _dot(xh, wqkv_v[:, D:2 * D]).astype(BF)
            kp = jnp.concatenate([k, jnp.zeros((TB1, 128), BF)], axis=1)
            for g in range(NG):
                k_s[g, r0:r0 + TB1, :] = kp[:, g * GW:g * GW + 128]
            v = _dot(xh, wqkv_v[:, 2 * D:3 * D])
            vt = v.T
            tail = (row32[0:12, :] == 0).astype(F32)
            for h in range(H):
                slot = jnp.concatenate([vt[h * DH:(h + 1) * DH, :], tail], axis=0)
                vt_s[h, :, r0:r0 + TB1] = slot.astype(BF)

        n = S // CK
        def attn_body(t, carry):
            qb = t // (H // HPB)
            hb = t - qb * (H // HPB)
            qsl = pl.ds(pl.multiple_of(qb * BQ, 128), BQ)
            qs = {}
            def get_q(i):
                if i not in qs:
                    g = hb * (HPB // G) + i // G
                    ii = i % G
                    q = qt_s[pl.ds(pl.multiple_of(g * GW, 16), 128), qsl]
                    row = lax.broadcasted_iota(jnp.int32, (128, BQ), 0)
                    q = jnp.where((row >= ii * DH) & (row < ii * DH + DH), q, jnp.zeros_like(q))
                    qs[i] = (g, q)
                return qs[i]
            def qk(idx):
                i, c = divmod(idx, n)
                g, q = get_q(i)
                return _dot(k_s[g, c * CK:(c + 1) * CK, :], q)
            total = HPB * n
            s = {0: qk(0)}
            o = None; m = None
            outs = []
            for idx in range(total):
                i, c = divmod(idx, n)
                if idx + 1 < total:
                    s[idx + 1] = qk(idx + 1)
                sc = s.pop(idx)
                if c == 0:
                    o = None; m = None
                mc = jnp.max(sc, axis=0, keepdims=True)
                m_new = mc if m is None else jnp.maximum(m, mc)
                p = jnp.exp2(sc - m_new).astype(BF)
                h = hb * HPB + i
                oc = _dot(vt_s[h, :, c * CK:(c + 1) * CK], p)
                o = oc if o is None else o * jnp.exp2(m - m_new) + oc
                m = m_new
                if c == n - 1:
                    inv = 1.0 / o[DH:DH + 1, :]
                    outs.append(o[0:DH, :] * inv)
                    if len(outs) == G:
                        g = hb * (HPB // G) + i // G
                        og = jnp.concatenate(outs, axis=0).astype(BF)
                        ot_s[pl.ds(pl.multiple_of(g * GW, 16), GW), qsl] = og
                        outs = []
            return carry
        lax.fori_loop(0, NQ * (H // HPB), attn_body, 0)

        wo_cp.wait(); w1_cp.wait(); w3_cp.wait(); w2_cp.wait()
        def out_cp(b, slot):
            return pltpu.make_async_copy(out_v.at[slot], out_hbm.at[pl.ds(b * TB3, TB3), :], sem_o.at[slot])
        nfc = (F + FC - 1) // FC
        def ffn_body(b, carry):
            r = pl.ds(pl.multiple_of(b * TB3, TB3), TB3)
            slot = b % 2
            ot = ot_s[:, r]
            a = lax.dot_general(ot, wo_v[...], (((0,), (0,)), ((), ())), preferred_element_type=F32)
            hres = x_v[r, :].astype(F32) + a
            hh = _ln(hres).astype(BF)
            def gu(c):
                lo = c * FC; hi = min(F, lo + FC)
                return _dot_nt(hh, w1_v[lo:hi, :]), _dot_nt(hh, w3_v[lo:hi, :])
            cur = gu(0)
            acc = None
            for c in range(nfc):
                nxt = gu(c + 1) if c + 1 < nfc else None
                gate, up = cur
                act = (gate * jax.nn.sigmoid(gate) * up).astype(BF)
                lo = c * FC; hi = min(F, lo + FC)
                dn = _dot(act, w2_v[lo:hi, :])
                acc = dn if acc is None else acc + dn
                cur = nxt
            res = (hres + acc).astype(BF)
            @pl.when(b >= 2)
            def _():
                out_cp(b - 2, slot).wait()
            out_v[slot] = res
            out_cp(b, slot).start()
            return carry
        lax.fori_loop(0, NB3, ffn_body, 0)
        out_cp(NB3 - 2, (NB3 - 2) % 2).wait()
        out_cp(NB3 - 1, (NB3 - 1) % 2).wait()

    scratch = [
        pltpu.VMEM((S, D), BF), pltpu.VMEM((D, 3 * D), BF), pltpu.VMEM((D, D), BF),
        pltpu.VMEM((F, D), BF), pltpu.VMEM((F, D), BF), pltpu.VMEM((F, D), BF),
        pltpu.VMEM((NG, S, 128), BF),
        pltpu.VMEM((D + 64, S), BF),
        pltpu.VMEM((H, 32, S), BF),
        pltpu.VMEM((D, S), BF),
        pltpu.VMEM((2, TB3, D), BF),
        pltpu.SemaphoreType.DMA((NXC,)),
        pltpu.SemaphoreType.DMA((7,)),
        pltpu.SemaphoreType.DMA((2,)),
    ]

    def fn(A_x, A_wqkv, A_wo, B_x, B_w1, B_w3, B_w2):
        anyspec = pl.BlockSpec(memory_space=pl.ANY)
        out = pl.pallas_call(
            kernel,
            out_shape=jax.ShapeDtypeStruct((S, D), BF),
            in_specs=[anyspec] * 6,
            out_specs=anyspec,
            scratch_shapes=scratch,
            compiler_params=pltpu.CompilerParams(vmem_limit_bytes=110 * 1024 * 1024),
            name=name,
        )(A_x.reshape(S, D), A_wqkv, A_wo, B_w1.T, B_w3.T, B_w2)
        return out.reshape(1, S, D)
    return fn


_kernel_fn = make_kernel(name="fused_block")


@jax.jit
def pallas_sequential_preLN__softmax_full_mha__glu_gated_swiglu__prompt_kernel(
    A_x, A_wqkv, A_wo, B_x, B_w1, B_w3, B_w2,
):
    return _kernel_fn(A_x, A_wqkv, A_wo, B_x, B_w1, B_w3, B_w2)
```

```python
import numpy as np
import jax
import jax.numpy as jnp
from jax import lax
import jax.experimental.pallas as pl
import jax.experimental.pallas.tpu as pltpu

S, D, H, DH, F = 2048, 640, 32, 20, 1728
G = 4
NG = H // G
GW = G * DH
VR = 24
EPS = 1e-5
QSCALE = float(DH ** -0.5 * np.log2(np.e))
BF = jnp.bfloat16
F32 = jnp.float32
FM = (F // 128) * 128
FR = F - FM

TB1 = 256
BQ = 1024
CK = 128
VK = 8
MK = CK - VK
P0 = 72
TB3 = 256
FC = 256
NQ = S // BQ
NT = NQ * NG
NB1 = S // TB1
X0 = 2 * TB1


def _ln(xf):
    m = jnp.mean(xf, axis=-1, keepdims=True)
    d = xf - m
    v = jnp.mean(d * d, axis=-1, keepdims=True)
    return d * lax.rsqrt(v + EPS)


def _dot(a, b):
    return lax.dot_general(a, b, (((1,), (0,)), ((), ())), preferred_element_type=F32)


def _dot_nt(a, b):
    return lax.dot_general(a, b, (((1,), (1,)), ((), ())), preferred_element_type=F32)


def _dot_tn(a, b):
    return lax.dot_general(a, b, (((0,), (0,)), ((), ())), preferred_element_type=F32)


def _p3_blocks():
    blocks = [(r, TB3) for r in range(0, S - TB3, TB3)]
    blocks += [(S - TB3, TB3 // 2), (S - TB3 // 2, TB3 // 2)]
    return blocks


def _kernel(x_hbm, wqkv_hbm, wo_hbm, w1t_hbm, w3t_hbm, w2_hbm, out_hbm,
            x_v, wqkv_v, wo_v, w1_v, w3_v, wr_v, w2_v,
            k_s, qt_s, vt_s, ot_s, qf_s, cy_s, h_s, hh_s, out_v, sem_x, sem_w, sem_o):
    x0_cp = pltpu.make_async_copy(x_hbm.at[pl.ds(0, X0), :], x_v.at[pl.ds(0, X0), :], sem_x.at[0])
    x1_cp = pltpu.make_async_copy(x_hbm.at[pl.ds(X0, S - X0), :], x_v.at[pl.ds(X0, S - X0), :], sem_x.at[1])

    def wqkv_cp(j):
        return pltpu.make_async_copy(wqkv_hbm.at[:, pl.ds(j * D, D)], wqkv_v.at[:, pl.ds(j * D, D)], sem_w.at[j])

    wo_cp = pltpu.make_async_copy(wo_hbm, wo_v, sem_w.at[3])
    w1_cp = pltpu.make_async_copy(w1t_hbm.at[pl.ds(0, FM), :], w1_v, sem_w.at[4])
    w3_cp = pltpu.make_async_copy(w3t_hbm.at[pl.ds(0, FM), :], w3_v, sem_w.at[5])
    w1r_cp = pltpu.make_async_copy(w1t_hbm.at[pl.ds(FM, FR), :], wr_v.at[pl.ds(0, FR), :], sem_w.at[6])
    w3r_cp = pltpu.make_async_copy(w3t_hbm.at[pl.ds(FM, FR), :], wr_v.at[pl.ds(FR, FR), :], sem_w.at[7])
    w2_cp = pltpu.make_async_copy(w2_hbm, w2_v, sem_w.at[8])
    x0_cp.start()
    wqkv_cp(0).start()

    qt_s[D:, :] = jnp.zeros((qt_s.shape[0] - D, S), BF)
    qf_s[:, :, GW:, :] = jnp.zeros((NQ, NG, 8, BQ), F32)

    ones_tail = (lax.broadcasted_iota(jnp.int32, (VR - DH, TB1), 0) == 0).astype(F32)
    xh = {}

    def ln1(b):
        r0 = b * TB1
        xh[b] = _ln(x_v[r0:r0 + TB1, :].astype(F32)).astype(BF)

    def qproj(b):
        r0 = b * TB1
        q = _dot(xh[b], wqkv_v[:, 0:D]) * QSCALE
        qtb = q.astype(BF).T
        qt_s[0:D, r0:r0 + TB1] = qtb
        qtf = qtb.astype(F32)
        for g in range(NG):
            qf_s[r0 // BQ, g, 0:GW, r0 % BQ:r0 % BQ + TB1] = qtf[g * GW:(g + 1) * GW, :]

    def kproj(b):
        r0 = b * TB1
        k = _dot(xh[b], wqkv_v[:, D:2 * D]).astype(BF)
        kp = jnp.concatenate([k, jnp.zeros((TB1, 128), BF)], axis=1)
        for g in range(NG):
            k_s[g, r0:r0 + TB1, :] = kp[:, g * GW:g * GW + 128].astype(F32)

    def vproj(b):
        r0 = b * TB1
        vt = _dot(xh[b], wqkv_v[:, 2 * D:3 * D]).T
        for h in range(H):
            vt_s[h, :, r0:r0 + TB1] = jnp.concatenate([vt[h * DH:(h + 1) * DH, :], ones_tail], axis=0)

    x0_cp.wait()
    wqkv_cp(1).start()
    ln1(0)
    ln1(1)
    wqkv_cp(0).wait()
    wqkv_cp(2).start()
    x1_cp.start()
    qproj(0)
    qproj(1)
    wqkv_cp(1).wait()
    kproj(0)
    kproj(1)
    wqkv_cp(2).wait()
    x1_cp.wait()
    vproj(0)
    ln1(2)
    vproj(1)
    for b in range(2, NB1):
        if b + 1 < NB1:
            ln1(b + 1)
        kproj(b)
        vproj(b)
        qproj(b)

    wo_cp.start()
    w1_cp.start()
    w3_cp.start()
    w1r_cp.start()
    w3r_cp.start()
    w2_cp.start()

    n = S // CK

    def masked_q(g, ii, qsl):
        q = qt_s[pl.ds(pl.multiple_of(g * GW, 16), 128), qsl]
        qi = pltpu.bitcast(q, jnp.int32)
        r2 = lax.broadcasted_iota(jnp.int32, (64, BQ), 0)
        qi = jnp.where((r2 >= ii * (DH // 2)) & (r2 < (ii + 1) * (DH // 2)), qi, 0)
        return pltpu.bitcast(qi, BF)

    def first_piece(t):
        qb = t // NG
        g = t - qb * NG
        qsl = pl.ds(pl.multiple_of(qb * BQ, 128), BQ)
        return _dot(k_s[g, 0:P0, :], masked_q(g, 0, qsl))

    def attn_body(t, carry):
        qb = t // NG
        g = t - qb * NG
        qsl = pl.ds(pl.multiple_of(qb * BQ, 128), BQ)
        qs = {}

        def get_q(i):
            if i not in qs:
                qs[i] = masked_q(g, i, qsl)
            return qs[i]

        def mxu_part(i, c):
            q = get_q(i)
            r0 = c * CK
            if i == 0 and c == 0:
                pa = cy_s[...]
            else:
                pa = _dot(k_s[g, r0:r0 + P0, :], q)
            pb = _dot(k_s[g, r0 + P0:r0 + MK, :], q)
            return jnp.concatenate([pa, pb], axis=0)

        def vpu_part(i, c):
            r0 = c * CK + MK
            kv = k_s[g, r0:r0 + VK, :]
            accs = [None, None]
            for d in range(DH):
                r = i * DH + d
                term = kv[:, r:r + 1] * qf_s[qb, g, pl.ds(r, 8, stride=0), :]
                accs[d % 2] = term if accs[d % 2] is None else accs[d % 2] + term
            return accs[0] + accs[1]

        total = G * n
        sm = {0: mxu_part(0, 0)}
        sv = {0: vpu_part(0, 0)}
        o = m = None
        outs = []
        for idx in range(total):
            i, c = divmod(idx, n)
            if idx + 1 < total:
                sm[idx + 1] = mxu_part(*divmod(idx + 1, n))
            else:
                cy_s[...] = first_piece(jnp.minimum(t + 1, NT - 1))
            if idx + 1 < total:
                sv[idx + 1] = vpu_part(*divmod(idx + 1, n))
            sc = jnp.concatenate([sm.pop(idx), sv.pop(idx)], axis=0)
            if c == 0:
                o = m = None
            mc = jnp.max(sc, axis=0, keepdims=True)
            m_new = mc if m is None else jnp.maximum(m, mc)
            p = jnp.exp2(sc - m_new).astype(BF)
            oc = _dot(vt_s[g * G + i, :, c * CK:(c + 1) * CK], p)
            o = oc if o is None else o * jnp.exp2(m - m_new) + oc
            m = m_new
            if c == n - 1:
                l = o[DH:DH + 1, :]
                inv = pl.reciprocal(l, approx=True)
                inv = inv * (2.0 - l * inv)
                outs.append(o[0:DH, :] * inv)
        og = jnp.concatenate(outs, axis=0).astype(BF)
        ot_s[pl.ds(pl.multiple_of(g * GW, 16), GW), qsl] = og
        return carry

    cy_s[...] = first_piece(0)
    lax.fori_loop(0, NT, attn_body, 0)

    wo_cp.wait()
    w1_cp.wait()
    w3_cp.wait()
    w1r_cp.wait()
    w3r_cp.wait()
    w2_cp.wait()
    blocks = _p3_blocks()
    chunks = [(lo, min(FM, lo + FC)) for lo in range(0, FM, FC)]
    nfc = len(chunks)

    def out_cp(b):
        r0, sz = blocks[b]
        return pltpu.make_async_copy(out_v.at[pl.ds(r0, sz), :], out_hbm.at[pl.ds(r0, sz), :], sem_o.at[b])

    def oproj_ln(b):
        r0, sz = blocks[b]
        a = _dot_tn(ot_s[:, r0:r0 + sz], wo_v[...])
        hres = x_v[r0:r0 + sz, :].astype(F32) + a
        h_s[r0:r0 + sz, :] = hres
        hh_s[r0:r0 + sz, :] = _ln(hres).astype(BF)

    def ffn(b):
        r0, sz = blocks[b]
        hh = hh_s[r0:r0 + sz, :]

        def gu(c):
            lo, hi = chunks[c]
            gate = _dot_nt(hh, w1_v[lo:hi, :])
            up = _dot_nt(hh, w3_v[lo:hi, :])
            rem = _dot_nt(hh, wr_v[...]) if c == nfc - 1 else None
            return gate, up, rem

        cur = gu(0)
        acc = None
        for c in range(nfc):
            nxt = gu(c + 1) if c + 1 < nfc else None
            if c == 3 and b + 1 < len(blocks):
                oproj_ln(b + 1)
            gate, up, rem = cur
            lo, hi = chunks[c]
            act = (gate * jax.nn.sigmoid(gate) * up).astype(BF)
            if rem is not None:
                ur = pltpu.roll(rem, FR, 1)
                ar = (rem * jax.nn.sigmoid(rem) * ur).astype(BF)[:, 0:FR]
                act = jnp.concatenate([act, ar], axis=1)
                hi = F
            dn = _dot(act, w2_v[lo:hi, :])
            acc = dn if acc is None else acc + dn
            cur = nxt
        out_v[r0:r0 + sz, :] = (h_s[r0:r0 + sz, :] + acc).astype(BF)
        out_cp(b).start()

    oproj_ln(0)
    for b in range(len(blocks)):
        ffn(b)
    for b in range(len(blocks)):
        out_cp(b).wait()


@jax.jit
def pallas_sequential_preLN__softmax_full_mha__glu_gated_swiglu__prompt_kernel(
    A_x: jax.Array,
    A_wqkv: jax.Array,
    A_wo: jax.Array,
    B_x: jax.Array,
    B_w1: jax.Array,
    B_w3: jax.Array,
    B_w2: jax.Array,
):
    del B_x
    scratch = [
        pltpu.VMEM((S, D), BF),
        pltpu.VMEM((D, 3 * D), BF),
        pltpu.VMEM((D, D), BF),
        pltpu.VMEM((FM, D), BF),
        pltpu.VMEM((FM, D), BF),
        pltpu.VMEM((2 * FR, D), BF),
        pltpu.VMEM((F, D), BF),
        pltpu.VMEM((NG, S, 128), F32),
        pltpu.VMEM((D + 64, S), BF),
        pltpu.VMEM((H, VR, S), F32),
        pltpu.VMEM((D, S), BF),
        pltpu.VMEM((NQ, NG, GW + 8, BQ), F32),
        pltpu.VMEM((P0, BQ), F32),
        pltpu.VMEM((S, D), F32),
        pltpu.VMEM((S, D), BF),
        pltpu.VMEM((S, D), BF),
        pltpu.SemaphoreType.DMA((2,)),
        pltpu.SemaphoreType.DMA((9,)),
        pltpu.SemaphoreType.DMA((len(_p3_blocks()),)),
    ]
    anyspec = pl.BlockSpec(memory_space=pl.ANY)
    out = pl.pallas_call(
        _kernel,
        out_shape=jax.ShapeDtypeStruct((S, D), BF),
        in_specs=[anyspec] * 6,
        out_specs=anyspec,
        scratch_shapes=scratch,
        compiler_params=pltpu.CompilerParams(vmem_limit_bytes=100 * 1024 * 1024),
        name="preln_mha_swiglu_block",
    )(A_x.reshape(S, D), A_wqkv, A_wo, B_w1.T, B_w3.T, B_w2)
    return out.reshape(1, S, D)
```

```python
import numpy as np
import jax
import jax.numpy as jnp
from jax import lax
import jax.experimental.pallas as pl
import jax.experimental.pallas.tpu as pltpu

S, D, H, DH, F = 2048, 640, 32, 20, 1728
G = 4
NG = H // G
GW = G * DH
VR = 24
EPS = 1e-5
QSCALE = float(DH ** -0.5 * np.log2(np.e))
BF = jnp.bfloat16
F32 = jnp.float32
FM = (F // 128) * 128
FR = F - FM

TB1 = 256
BQ = 1024
CK = 128
VK = 8
MK = CK - VK
P0 = 72
TB3 = 256
FC = 256
NQ = S // BQ
NT = NQ * NG
NB1 = S // TB1
X0 = 2 * TB1


def _ln(xf):
    m = jnp.mean(xf, axis=-1, keepdims=True)
    d = xf - m
    v = jnp.mean(d * d, axis=-1, keepdims=True)
    return d * lax.rsqrt(v + EPS)


def _dot(a, b):
    return lax.dot_general(a, b, (((1,), (0,)), ((), ())), preferred_element_type=F32)


def _dot_nt(a, b):
    return lax.dot_general(a, b, (((1,), (1,)), ((), ())), preferred_element_type=F32)


def _dot_tn(a, b):
    return lax.dot_general(a, b, (((0,), (0,)), ((), ())), preferred_element_type=F32)


def _p3_blocks():
    blocks = [(r, TB3) for r in range(0, S - TB3, TB3)]
    blocks += [(S - TB3, TB3 // 2), (S - TB3 // 2, TB3 // 2)]
    return blocks


def _kernel(x_hbm, wqkv_hbm, wo_hbm, w1t_hbm, w3t_hbm, w2_hbm, out_hbm,
            x_v, wqkv_v, wo_v, w1_v, w3_v, wr_v, w2_v,
            k_s, qt_s, vt_s, ot_s, qf_s, qb_s, cy_s, h_s, hh_s, out_v, sem_x, sem_w, sem_o):
    x0_cp = pltpu.make_async_copy(x_hbm.at[pl.ds(0, X0), :], x_v.at[pl.ds(0, X0), :], sem_x.at[0])
    x1_cp = pltpu.make_async_copy(x_hbm.at[pl.ds(X0, S - X0), :], x_v.at[pl.ds(X0, S - X0), :], sem_x.at[1])

    def wqkv_cp(j):
        return pltpu.make_async_copy(wqkv_hbm.at[:, pl.ds(j * D, D)], wqkv_v.at[:, pl.ds(j * D, D)], sem_w.at[j])

    wo_cp = pltpu.make_async_copy(wo_hbm, wo_v, sem_w.at[3])
    w1_cp = pltpu.make_async_copy(w1t_hbm.at[pl.ds(0, FM), :], w1_v, sem_w.at[4])
    w3_cp = pltpu.make_async_copy(w3t_hbm.at[pl.ds(0, FM), :], w3_v, sem_w.at[5])
    w1r_cp = pltpu.make_async_copy(w1t_hbm.at[pl.ds(FM, FR), :], wr_v.at[pl.ds(0, FR), :], sem_w.at[6])
    w3r_cp = pltpu.make_async_copy(w3t_hbm.at[pl.ds(FM, FR), :], wr_v.at[pl.ds(FR, FR), :], sem_w.at[7])
    w2_cp = pltpu.make_async_copy(w2_hbm, w2_v, sem_w.at[8])
    x0_cp.start()
    wqkv_cp(0).start()

    qt_s[D:, :] = jnp.zeros((qt_s.shape[0] - D, S), BF)

    ones_tail = (lax.broadcasted_iota(jnp.int32, (VR - DH, TB1), 0) == 0).astype(F32)
    xh = {}

    def ln1(b):
        r0 = b * TB1
        xh[b] = _ln(x_v[r0:r0 + TB1, :].astype(F32)).astype(BF)

    def qproj(b):
        r0 = b * TB1
        q = _dot(xh[b], wqkv_v[:, 0:D]) * QSCALE
        qtb = q.astype(BF).T
        qt_s[0:D, r0:r0 + TB1] = qtb
        qtf = qtb.astype(F32)
        for g in range(NG):
            qf_s[r0 // BQ, g, :, r0 % BQ:r0 % BQ + TB1] = qtf[g * GW:(g + 1) * GW, :]

    def kproj(b):
        r0 = b * TB1
        k = _dot(xh[b], wqkv_v[:, D:2 * D]).astype(BF)
        kp = jnp.concatenate([k, jnp.zeros((TB1, 128), BF)], axis=1)
        for g in range(NG):
            k_s[g, r0:r0 + TB1, :] = kp[:, g * GW:g * GW + 128].astype(F32)

    def vproj(b):
        r0 = b * TB1
        vt = _dot(xh[b], wqkv_v[:, 2 * D:3 * D]).T
        for h in range(H):
            vt_s[h, :, r0:r0 + TB1] = jnp.concatenate([vt[h * DH:(h + 1) * DH, :], ones_tail], axis=0)

    x0_cp.wait()
    wqkv_cp(1).start()
    wqkv_cp(2).start()
    ln1(0)
    ln1(1)
    wqkv_cp(0).wait()
    x1_cp.start()
    qproj(0)
    qproj(1)
    wqkv_cp(1).wait()
    kproj(0)
    kproj(1)
    wqkv_cp(2).wait()
    x1_cp.wait()
    vproj(0)
    ln1(2)
    vproj(1)
    for b in range(2, NB1):
        if b + 1 < NB1:
            ln1(b + 1)
        qproj(b)
        vproj(b)
        kproj(b)

    wo_cp.start()
    w1_cp.start()
    w3_cp.start()
    w1r_cp.start()
    w3r_cp.start()
    w2_cp.start()

    n = S // CK

    def masked_q(g, ii, qsl):
        q = qt_s[pl.ds(pl.multiple_of(g * GW, 16), 128), qsl]
        qi = pltpu.bitcast(q, jnp.int32)
        r2 = lax.broadcasted_iota(jnp.int32, (64, BQ), 0)
        qi = jnp.where((r2 >= ii * (DH // 2)) & (r2 < (ii + 1) * (DH // 2)), qi, 0)
        return pltpu.bitcast(qi, BF)

    def first_piece(t):
        qb = t // NG
        g = t - qb * NG
        qsl = pl.ds(pl.multiple_of(qb * BQ, 128), BQ)
        return _dot(k_s[g, 0:P0, :], masked_q(g, 0, qsl))

    def spread_q(t, i):
        qb = t // NG
        g = t - qb * NG
        for d in range(DH):
            r = i * DH + d
            qb_s[i % 2, d] = jnp.broadcast_to(qf_s[qb, g, r:r + 1, :], (8, BQ))

    def attn_body(t, carry):
        qb = t // NG
        g = t - qb * NG
        qsl = pl.ds(pl.multiple_of(qb * BQ, 128), BQ)
        qs = {}

        def get_q(i):
            if i not in qs:
                qs[i] = masked_q(g, i, qsl)
            return qs[i]

        def mxu_part(i, c):
            q = get_q(i)
            r0 = c * CK
            if i == 0 and c == 0:
                pa = cy_s[...]
            else:
                pa = _dot(k_s[g, r0:r0 + P0, :], q)
            pb = _dot(k_s[g, r0 + P0:r0 + MK, :], q)
            return jnp.concatenate([pa, pb], axis=0)

        def vpu_part(i, c):
            r0 = c * CK + MK
            kv = k_s[g, r0:r0 + VK, :]
            accs = [None, None]
            for d in range(DH):
                r = i * DH + d
                term = kv[:, r:r + 1] * qb_s[i % 2, d]
                accs[d % 2] = term if accs[d % 2] is None else accs[d % 2] + term
            return accs[0] + accs[1]

        total = G * n
        sm = {0: mxu_part(0, 0)}
        sv = {0: vpu_part(0, 0)}
        o = m = None
        outs = []
        for idx in range(total):
            i, c = divmod(idx, n)
            if idx + 1 < total:
                sm[idx + 1] = mxu_part(*divmod(idx + 1, n))
            else:
                cy_s[...] = first_piece(jnp.minimum(t + 1, NT - 1))
            if c == n - 1:
                if i + 1 < G:
                    spread_q(t, i + 1)
                else:
                    spread_q(jnp.minimum(t + 1, NT - 1), 0)
            if idx + 1 < total:
                sv[idx + 1] = vpu_part(*divmod(idx + 1, n))
            sc = jnp.concatenate([sm.pop(idx), sv.pop(idx)], axis=0)
            if c == 0:
                o = m = None
            mc = jnp.max(sc, axis=0, keepdims=True)
            m_new = mc if m is None else jnp.maximum(m, mc)
            p = jnp.exp2(sc - m_new).astype(BF)
            oc = _dot(vt_s[g * G + i, :, c * CK:(c + 1) * CK], p)
            o = oc if o is None else o * jnp.exp2(m - m_new) + oc
            m = m_new
            if c == n - 1:
                l = o[DH:DH + 1, :]
                inv = pl.reciprocal(l, approx=True)
                inv = inv * (2.0 - l * inv)
                outs.append(o[0:DH, :] * inv)
        og = jnp.concatenate(outs, axis=0).astype(BF)
        ot_s[pl.ds(pl.multiple_of(g * GW, 16), GW), qsl] = og
        return carry

    cy_s[...] = first_piece(0)
    spread_q(0, 0)
    lax.fori_loop(0, NT, attn_body, 0)

    wo_cp.wait()
    w1_cp.wait()
    w3_cp.wait()
    w1r_cp.wait()
    w3r_cp.wait()
    w2_cp.wait()
    blocks = _p3_blocks()
    chunks = [(lo, min(FM, lo + FC)) for lo in range(0, FM, FC)]
    nfc = len(chunks)

    def out_cp(b):
        r0, sz = blocks[b]
        return pltpu.make_async_copy(out_v.at[pl.ds(r0, sz), :], out_hbm.at[pl.ds(r0, sz), :], sem_o.at[b])

    def oproj_ln(b):
        r0, sz = blocks[b]
        a = _dot_tn(ot_s[:, r0:r0 + sz], wo_v[...])
        hres = x_v[r0:r0 + sz, :].astype(F32) + a
        h_s[r0:r0 + sz, :] = hres
        hh_s[r0:r0 + sz, :] = _ln(hres).astype(BF)

    def ffn(b):
        r0, sz = blocks[b]
        hh = hh_s[r0:r0 + sz, :]

        def gu(c):
            lo, hi = chunks[c]
            gate = _dot_nt(hh, w1_v[lo:hi, :])
            up = _dot_nt(hh, w3_v[lo:hi, :])
            rem = _dot_nt(hh, wr_v[...]) if c == nfc - 1 else None
            return gate, up, rem

        cur = gu(0)
        acc = None
        for c in range(nfc):
            nxt = gu(c + 1) if c + 1 < nfc else None
            if c == 2 and b + 1 < len(blocks):
                oproj_ln(b + 1)
            gate, up, rem = cur
            lo, hi = chunks[c]
            act = (gate * jax.nn.sigmoid(gate) * up).astype(BF)
            if rem is not None:
                ur = pltpu.roll(rem, FR, 1)
                ar = (rem * jax.nn.sigmoid(rem) * ur).astype(BF)[:, 0:FR]
                act = jnp.concatenate([act, ar], axis=1)
                hi = F
            dn = _dot(act, w2_v[lo:hi, :])
            acc = dn if acc is None else acc + dn
            cur = nxt
        out_v[r0:r0 + sz, :] = (h_s[r0:r0 + sz, :] + acc).astype(BF)
        out_cp(b).start()

    oproj_ln(0)
    for b in range(len(blocks)):
        ffn(b)
    for b in range(len(blocks)):
        out_cp(b).wait()


@jax.jit
def pallas_sequential_preLN__softmax_full_mha__glu_gated_swiglu__prompt_kernel(
    A_x: jax.Array,
    A_wqkv: jax.Array,
    A_wo: jax.Array,
    B_x: jax.Array,
    B_w1: jax.Array,
    B_w3: jax.Array,
    B_w2: jax.Array,
):
    del B_x
    scratch = [
        pltpu.VMEM((S, D), BF),
        pltpu.VMEM((D, 3 * D), BF),
        pltpu.VMEM((D, D), BF),
        pltpu.VMEM((FM, D), BF),
        pltpu.VMEM((FM, D), BF),
        pltpu.VMEM((2 * FR, D), BF),
        pltpu.VMEM((F, D), BF),
        pltpu.VMEM((NG, S, 128), F32),
        pltpu.VMEM((D + 64, S), BF),
        pltpu.VMEM((H, VR, S), F32),
        pltpu.VMEM((D, S), BF),
        pltpu.VMEM((NQ, NG, GW, BQ), F32),
        pltpu.VMEM((2, DH, 8, BQ), F32),
        pltpu.VMEM((P0, BQ), F32),
        pltpu.VMEM((S, D), F32),
        pltpu.VMEM((S, D), BF),
        pltpu.VMEM((S, D), BF),
        pltpu.SemaphoreType.DMA((2,)),
        pltpu.SemaphoreType.DMA((9,)),
        pltpu.SemaphoreType.DMA((len(_p3_blocks()),)),
    ]
    anyspec = pl.BlockSpec(memory_space=pl.ANY)
    out = pl.pallas_call(
        _kernel,
        out_shape=jax.ShapeDtypeStruct((S, D), BF),
        in_specs=[anyspec] * 6,
        out_specs=anyspec,
        scratch_shapes=scratch,
        compiler_params=pltpu.CompilerParams(vmem_limit_bytes=100 * 1024 * 1024),
        name="preln_mha_swiglu_block",
    )(A_x.reshape(S, D), A_wqkv, A_wo, B_w1.T, B_w3.T, B_w2)
    return out.reshape(1, S, D)
```

```python
import numpy as np
import jax
import jax.numpy as jnp
from jax import lax
import jax.experimental.pallas as pl
import jax.experimental.pallas.tpu as pltpu

S, D, H, DH, F = 2048, 640, 32, 20, 1728
G = 4
NG = H // G
GW = G * DH
VR = 24
EPS = 1e-5
QSCALE = float(DH ** -0.5 * np.log2(np.e))
BF = jnp.bfloat16
F32 = jnp.float32
FM = (F // 128) * 128
FR = F - FM

TB1 = 256
BQ = 1024
CK = 128
VK = 8
MK = CK - VK
P0 = 72
TB3 = 256
FC = 256
NQ = S // BQ
NT = NQ * NG
NB1 = S // TB1
X0 = 2 * TB1


def _ln(xf):
    m = jnp.mean(xf, axis=-1, keepdims=True)
    d = xf - m
    v = jnp.mean(d * d, axis=-1, keepdims=True)
    return d * lax.rsqrt(v + EPS)


def _dot(a, b):
    return lax.dot_general(a, b, (((1,), (0,)), ((), ())), preferred_element_type=F32)


def _dot_nt(a, b):
    return lax.dot_general(a, b, (((1,), (1,)), ((), ())), preferred_element_type=F32)


def _dot_tn(a, b):
    return lax.dot_general(a, b, (((0,), (0,)), ((), ())), preferred_element_type=F32)


def _p3_blocks():
    blocks = [(r, TB3) for r in range(0, S - TB3, TB3)]
    blocks += [(S - TB3, TB3 // 2), (S - TB3 // 2, TB3 // 2)]
    return blocks


def _kernel(x_hbm, wqkv_hbm, wo_hbm, w1t_hbm, w3t_hbm, w2_hbm, out_hbm,
            x_v, wqkv_v, wo_v, w1_v, w3_v, wr_v, w2_v,
            k_s, qt_s, vt_s, ot_s, qr_s, cy_s, h_s, hh_s, out_v, sem_x, sem_w, sem_o):
    x0_cp = pltpu.make_async_copy(x_hbm.at[pl.ds(0, X0), :], x_v.at[pl.ds(0, X0), :], sem_x.at[0])
    x1_cp = pltpu.make_async_copy(x_hbm.at[pl.ds(X0, S - X0), :], x_v.at[pl.ds(X0, S - X0), :], sem_x.at[1])

    def wqkv_cp(j):
        return pltpu.make_async_copy(wqkv_hbm.at[:, pl.ds(j * D, D)], wqkv_v.at[:, pl.ds(j * D, D)], sem_w.at[j])

    wo_cp = pltpu.make_async_copy(wo_hbm, wo_v, sem_w.at[3])
    w1_cp = pltpu.make_async_copy(w1t_hbm.at[pl.ds(0, FM), :], w1_v, sem_w.at[4])
    w3_cp = pltpu.make_async_copy(w3t_hbm.at[pl.ds(0, FM), :], w3_v, sem_w.at[5])
    w1r_cp = pltpu.make_async_copy(w1t_hbm.at[pl.ds(FM, FR), :], wr_v.at[pl.ds(0, FR), :], sem_w.at[6])
    w3r_cp = pltpu.make_async_copy(w3t_hbm.at[pl.ds(FM, FR), :], wr_v.at[pl.ds(FR, FR), :], sem_w.at[7])
    w2_cp = pltpu.make_async_copy(w2_hbm, w2_v, sem_w.at[8])
    x0_cp.start()
    wqkv_cp(0).start()

    qt_s[D:, :] = jnp.zeros((qt_s.shape[0] - D, S), BF)

    ones_tail = (lax.broadcasted_iota(jnp.int32, (VR - DH, TB1), 0) == 0).astype(F32)
    xh = {}

    def ln1(b):
        r0 = b * TB1
        xh[b] = _ln(x_v[r0:r0 + TB1, :].astype(F32)).astype(BF)

    def qproj(b):
        r0 = b * TB1
        q = _dot(xh[b], wqkv_v[:, 0:D]) * QSCALE
        qtb = q.astype(BF).T
        qt_s[0:D, r0:r0 + TB1] = qtb
        if b >= 2:
            spread_q(b, qtb)

    def spread_q(b, qtb=None):
        r0 = b * TB1
        for g in range(NG):
            if qtb is None:
                qtf = qt_s[g * GW:(g + 1) * GW, r0:r0 + TB1].astype(F32)
            else:
                qtf = qtb[g * GW:(g + 1) * GW, :].astype(F32)
            for r in range(GW):
                qr_s[r0 // BQ, g, r, :, r0 % BQ:r0 % BQ + TB1] = jnp.broadcast_to(qtf[r:r + 1, :], (8, TB1))

    def kproj(b):
        r0 = b * TB1
        k = _dot(xh[b], wqkv_v[:, D:2 * D]).astype(BF)
        kp = jnp.concatenate([k, jnp.zeros((TB1, 128), BF)], axis=1)
        for g in range(NG):
            k_s[g, r0:r0 + TB1, :] = kp[:, g * GW:g * GW + 128].astype(F32)

    def vproj(b):
        r0 = b * TB1
        vt = _dot(xh[b], wqkv_v[:, 2 * D:3 * D]).T
        for h in range(H):
            vt_s[h, :, r0:r0 + TB1] = jnp.concatenate([vt[h * DH:(h + 1) * DH, :], ones_tail], axis=0)

    x0_cp.wait()
    wqkv_cp(1).start()
    wqkv_cp(2).start()
    ln1(0)
    ln1(1)
    wqkv_cp(0).wait()
    x1_cp.start()
    qproj(0)
    qproj(1)
    wqkv_cp(1).wait()
    kproj(0)
    spread_q(0)
    kproj(1)
    wqkv_cp(2).wait()
    x1_cp.wait()
    vproj(0)
    ln1(2)
    spread_q(1)
    vproj(1)
    for b in range(2, NB1):
        if b + 1 < NB1:
            ln1(b + 1)
        qproj(b)
        vproj(b)
        kproj(b)

    wo_cp.start()
    w1_cp.start()
    w3_cp.start()
    w1r_cp.start()
    w3r_cp.start()
    w2_cp.start()

    n = S // CK

    def masked_q(g, ii, qsl):
        q = qt_s[pl.ds(pl.multiple_of(g * GW, 16), 128), qsl]
        qi = pltpu.bitcast(q, jnp.int32)
        r2 = lax.broadcasted_iota(jnp.int32, (64, BQ), 0)
        qi = jnp.where((r2 >= ii * (DH // 2)) & (r2 < (ii + 1) * (DH // 2)), qi, 0)
        return pltpu.bitcast(qi, BF)

    def first_piece(t):
        qb = t // NG
        g = t - qb * NG
        qsl = pl.ds(pl.multiple_of(qb * BQ, 128), BQ)
        return _dot(k_s[g, 0:P0, :], masked_q(g, 0, qsl))

    def attn_body(t, carry):
        qb = t // NG
        g = t - qb * NG
        qsl = pl.ds(pl.multiple_of(qb * BQ, 128), BQ)
        qs = {}

        def get_q(i):
            if i not in qs:
                qs[i] = masked_q(g, i, qsl)
            return qs[i]

        def mxu_part(i, c):
            q = get_q(i)
            r0 = c * CK
            if i == 0 and c == 0:
                pa = cy_s[...]
            else:
                pa = _dot(k_s[g, r0:r0 + P0, :], q)
            pb = _dot(k_s[g, r0 + P0:r0 + MK, :], q)
            return jnp.concatenate([pa, pb], axis=0)

        def vpu_part(i, c):
            r0 = c * CK + MK
            kv = k_s[g, r0:r0 + VK, :]
            accs = [None, None]
            for d in range(DH):
                r = i * DH + d
                term = kv[:, r:r + 1] * qr_s[qb, g, r]
                accs[d % 2] = term if accs[d % 2] is None else accs[d % 2] + term
            return accs[0] + accs[1]

        total = G * n
        sm = {0: mxu_part(0, 0)}
        sv = {0: vpu_part(0, 0)}
        o = m = None
        outs = []
        for idx in range(total):
            i, c = divmod(idx, n)
            if idx + 1 < total:
                sm[idx + 1] = mxu_part(*divmod(idx + 1, n))
            else:
                cy_s[...] = first_piece(jnp.minimum(t + 1, NT - 1))
            if idx + 1 < total:
                sv[idx + 1] = vpu_part(*divmod(idx + 1, n))
            sc = jnp.concatenate([sm.pop(idx), sv.pop(idx)], axis=0)
            if c == 0:
                o = m = None
            mc = jnp.max(sc, axis=0, keepdims=True)
            m_new = mc if m is None else jnp.maximum(m, mc)
            p = jnp.exp2(sc - m_new).astype(BF)
            oc = _dot(vt_s[g * G + i, :, c * CK:(c + 1) * CK], p)
            o = oc if o is None else o * jnp.exp2(m - m_new) + oc
            m = m_new
            if c == n - 1:
                l = o[DH:DH + 1, :]
                inv = pl.reciprocal(l, approx=True)
                inv = inv * (2.0 - l * inv)
                outs.append(o[0:DH, :] * inv)
        og = jnp.concatenate(outs, axis=0).astype(BF)
        ot_s[pl.ds(pl.multiple_of(g * GW, 16), GW), qsl] = og
        return carry

    cy_s[...] = first_piece(0)
    lax.fori_loop(0, NT, attn_body, 0)

    wo_cp.wait()
    w1_cp.wait()
    w3_cp.wait()
    w1r_cp.wait()
    w3r_cp.wait()
    w2_cp.wait()
    blocks = _p3_blocks()
    chunks = [(lo, min(FM, lo + FC)) for lo in range(0, FM, FC)]
    nfc = len(chunks)

    def out_cp(b):
        r0, sz = blocks[b]
        return pltpu.make_async_copy(out_v.at[pl.ds(r0, sz), :], out_hbm.at[pl.ds(r0, sz), :], sem_o.at[b])

    def oproj_ln(b):
        r0, sz = blocks[b]
        a = _dot_tn(ot_s[:, r0:r0 + sz], wo_v[...])
        hres = x_v[r0:r0 + sz, :].astype(F32) + a
        h_s[r0:r0 + sz, :] = hres
        hh_s[r0:r0 + sz, :] = _ln(hres).astype(BF)

    def ffn(b):
        r0, sz = blocks[b]
        hh = hh_s[r0:r0 + sz, :]

        def gu(c):
            lo, hi = chunks[c]
            gate = _dot_nt(hh, w1_v[lo:hi, :])
            up = _dot_nt(hh, w3_v[lo:hi, :])
            rem = _dot_nt(hh, wr_v[...]) if c == nfc - 1 else None
            return gate, up, rem

        cur = gu(0)
        acc = None
        for c in range(nfc):
            nxt = gu(c + 1) if c + 1 < nfc else None
            if c == 2 and b + 1 < len(blocks):
                oproj_ln(b + 1)
            gate, up, rem = cur
            lo, hi = chunks[c]
            act = (gate * jax.nn.sigmoid(gate) * up).astype(BF)
            if rem is not None:
                ur = pltpu.roll(rem, FR, 1)
                ar = (rem * jax.nn.sigmoid(rem) * ur).astype(BF)[:, 0:FR]
                act = jnp.concatenate([act, ar], axis=1)
                hi = F
            dn = _dot(act, w2_v[lo:hi, :])
            acc = dn if acc is None else acc + dn
            cur = nxt
        out_v[r0:r0 + sz, :] = (h_s[r0:r0 + sz, :] + acc).astype(BF)
        out_cp(b).start()

    oproj_ln(0)
    for b in range(len(blocks)):
        ffn(b)
    for b in range(len(blocks)):
        out_cp(b).wait()


@jax.jit
def pallas_sequential_preLN__softmax_full_mha__glu_gated_swiglu__prompt_kernel(
    A_x: jax.Array,
    A_wqkv: jax.Array,
    A_wo: jax.Array,
    B_x: jax.Array,
    B_w1: jax.Array,
    B_w3: jax.Array,
    B_w2: jax.Array,
):
    del B_x
    scratch = [
        pltpu.VMEM((S, D), BF),
        pltpu.VMEM((D, 3 * D), BF),
        pltpu.VMEM((D, D), BF),
        pltpu.VMEM((FM, D), BF),
        pltpu.VMEM((FM, D), BF),
        pltpu.VMEM((2 * FR, D), BF),
        pltpu.VMEM((F, D), BF),
        pltpu.VMEM((NG, S, 128), F32),
        pltpu.VMEM((D + 64, S), BF),
        pltpu.VMEM((H, VR, S), F32),
        pltpu.VMEM((D, S), BF),
        pltpu.VMEM((NQ, NG, GW, 8, BQ), F32),
        pltpu.VMEM((P0, BQ), F32),
        pltpu.VMEM((S, D), F32),
        pltpu.VMEM((S, D), BF),
        pltpu.VMEM((S, D), BF),
        pltpu.SemaphoreType.DMA((2,)),
        pltpu.SemaphoreType.DMA((9,)),
        pltpu.SemaphoreType.DMA((len(_p3_blocks()),)),
    ]
    anyspec = pl.BlockSpec(memory_space=pl.ANY)
    out = pl.pallas_call(
        _kernel,
        out_shape=jax.ShapeDtypeStruct((S, D), BF),
        in_specs=[anyspec] * 6,
        out_specs=anyspec,
        scratch_shapes=scratch,
        compiler_params=pltpu.CompilerParams(vmem_limit_bytes=112 * 1024 * 1024),
        name="preln_mha_swiglu_block",
    )(A_x.reshape(S, D), A_wqkv, A_wo, B_w1.T, B_w3.T, B_w2)
    return out.reshape(1, S, D)
```

```python
import numpy as np
import jax
import jax.numpy as jnp
from jax import lax
import jax.experimental.pallas as pl
import jax.experimental.pallas.tpu as pltpu

S, D, H, DH, F = 2048, 640, 32, 20, 1728
G = 4
NG = H // G
GW = G * DH
VR = 24
EPS = 1e-5
QSCALE = float(DH ** -0.5 * np.log2(np.e))
BF = jnp.bfloat16
F32 = jnp.float32
FM = (F // 128) * 128
FR = F - FM

TB1 = 256
BQ = 1024
CK = 128
VK = 8
MK = CK - VK
P0 = 72
TB3 = 256
FC = 256
NQ = S // BQ
NT = NQ * NG
NB1 = S // TB1
X0 = 2 * TB1


def _ln(xf):
    m = jnp.mean(xf, axis=-1, keepdims=True)
    d = xf - m
    v = jnp.mean(d * d, axis=-1, keepdims=True)
    return d * lax.rsqrt(v + EPS)


def _dot(a, b):
    return lax.dot_general(a, b, (((1,), (0,)), ((), ())), preferred_element_type=F32)


def _dot_nt(a, b):
    return lax.dot_general(a, b, (((1,), (1,)), ((), ())), preferred_element_type=F32)


def _dot_tn(a, b):
    return lax.dot_general(a, b, (((0,), (0,)), ((), ())), preferred_element_type=F32)


def _p3_blocks():
    blocks = [(r, TB3) for r in range(0, S - TB3, TB3)]
    blocks += [(S - TB3, TB3 // 2), (S - TB3 // 2, TB3 // 2)]
    return blocks


def _kernel(x_hbm, wqkv_hbm, wo_hbm, w1t_hbm, w3t_hbm, w2_hbm, out_hbm,
            x_v, wqkv_v, wo_v, w1_v, w3_v, wr_v, w2_v,
            k_s, qt_s, vt_s, ot_s, qr_s, cy_s, h_s, hh_s, out_v, sem_x, sem_w, sem_o):
    x0_cp = pltpu.make_async_copy(x_hbm.at[pl.ds(0, X0), :], x_v.at[pl.ds(0, X0), :], sem_x.at[0])
    x1_cp = pltpu.make_async_copy(x_hbm.at[pl.ds(X0, S - X0), :], x_v.at[pl.ds(X0, S - X0), :], sem_x.at[1])

    def wqkv_cp(j):
        return pltpu.make_async_copy(wqkv_hbm.at[:, pl.ds(j * D, D)], wqkv_v.at[:, pl.ds(j * D, D)], sem_w.at[j])

    wo_cp = pltpu.make_async_copy(wo_hbm, wo_v, sem_w.at[3])
    w1_cp = pltpu.make_async_copy(w1t_hbm.at[pl.ds(0, FM), :], w1_v, sem_w.at[4])
    w3_cp = pltpu.make_async_copy(w3t_hbm.at[pl.ds(0, FM), :], w3_v, sem_w.at[5])
    w1r_cp = pltpu.make_async_copy(w1t_hbm.at[pl.ds(FM, FR), :], wr_v.at[pl.ds(0, FR), :], sem_w.at[6])
    w3r_cp = pltpu.make_async_copy(w3t_hbm.at[pl.ds(FM, FR), :], wr_v.at[pl.ds(FR, FR), :], sem_w.at[7])
    w2_cp = pltpu.make_async_copy(w2_hbm, w2_v, sem_w.at[8])
    x0_cp.start()
    wqkv_cp(1).start()

    qt_s[D:, :] = jnp.zeros((qt_s.shape[0] - D, S), BF)

    ones_tail = (lax.broadcasted_iota(jnp.int32, (VR - DH, TB1), 0) == 0).astype(F32)
    xh = {}

    def ln1(b):
        r0 = b * TB1
        xh[b] = _ln(x_v[r0:r0 + TB1, :].astype(F32)).astype(BF)

    def qproj(b):
        r0 = b * TB1
        q = _dot(xh[b], wqkv_v[:, 0:D]) * QSCALE
        qtb = q.astype(BF).T
        qt_s[0:D, r0:r0 + TB1] = qtb
        spread_q(b, qtb)

    def spread_q(b, qtb=None):
        r0 = b * TB1
        for g in range(NG):
            if qtb is None:
                qtf = qt_s[g * GW:(g + 1) * GW, r0:r0 + TB1].astype(F32)
            else:
                qtf = qtb[g * GW:(g + 1) * GW, :].astype(F32)
            for r in range(GW):
                qr_s[r0 // BQ, g, r, :, r0 % BQ:r0 % BQ + TB1] = jnp.broadcast_to(qtf[r:r + 1, :], (8, TB1))

    def kproj(b):
        r0 = b * TB1
        k = _dot(xh[b], wqkv_v[:, D:2 * D]).astype(BF)
        kp = jnp.concatenate([k, jnp.zeros((TB1, 128), BF)], axis=1)
        for g in range(NG):
            k_s[g, r0:r0 + TB1, :] = kp[:, g * GW:g * GW + 128].astype(F32)

    def vproj(b):
        r0 = b * TB1
        vt = _dot(xh[b], wqkv_v[:, 2 * D:3 * D]).T
        for h in range(H):
            vt_s[h, :, r0:r0 + TB1] = jnp.concatenate([vt[h * DH:(h + 1) * DH, :], ones_tail], axis=0)

    x0_cp.wait()
    wqkv_cp(2).start()
    wqkv_cp(0).start()
    ln1(0)
    ln1(1)
    wqkv_cp(1).wait()
    x1_cp.start()
    kproj(0)
    kproj(1)
    wqkv_cp(2).wait()
    wqkv_cp(0).wait()
    qproj(0)
    vproj(0)
    x1_cp.wait()
    ln1(2)
    qproj(1)
    vproj(1)
    for b in range(2, NB1):
        if b + 1 < NB1:
            ln1(b + 1)
        qproj(b)
        vproj(b)
        kproj(b)

    wo_cp.start()
    w1_cp.start()
    w3_cp.start()
    w1r_cp.start()
    w3r_cp.start()
    w2_cp.start()

    n = S // CK

    def masked_q(g, ii, qsl):
        q = qt_s[pl.ds(pl.multiple_of(g * GW, 16), 128), qsl]
        qi = pltpu.bitcast(q, jnp.int32)
        r2 = lax.broadcasted_iota(jnp.int32, (64, BQ), 0)
        qi = jnp.where((r2 >= ii * (DH // 2)) & (r2 < (ii + 1) * (DH // 2)), qi, 0)
        return pltpu.bitcast(qi, BF)

    def first_piece(t):
        qb = t // NG
        g = t - qb * NG
        qsl = pl.ds(pl.multiple_of(qb * BQ, 128), BQ)
        return _dot(k_s[g, 0:P0, :], masked_q(g, 0, qsl))

    def attn_body(t, carry):
        qb = t // NG
        g = t - qb * NG
        qsl = pl.ds(pl.multiple_of(qb * BQ, 128), BQ)
        qs = {}

        def get_q(i):
            if i not in qs:
                qs[i] = masked_q(g, i, qsl)
            return qs[i]

        def mxu_part(i, c):
            q = get_q(i)
            r0 = c * CK
            if i == 0 and c == 0:
                pa = cy_s[...]
            else:
                pa = _dot(k_s[g, r0:r0 + P0, :], q)
            pb = _dot(k_s[g, r0 + P0:r0 + MK, :], q)
            return jnp.concatenate([pa, pb], axis=0)

        def vpu_part(i, c):
            r0 = c * CK + MK
            kv = k_s[g, r0:r0 + VK, :]
            accs = [None, None]
            for d in range(DH):
                r = i * DH + d
                term = kv[:, r:r + 1] * qr_s[qb, g, r]
                accs[d % 2] = term if accs[d % 2] is None else accs[d % 2] + term
            return accs[0] + accs[1]

        total = G * n
        sm = {0: mxu_part(0, 0)}
        sv = {0: vpu_part(0, 0)}
        o = m = None
        outs = []
        for idx in range(total):
            i, c = divmod(idx, n)
            if idx + 1 < total:
                sm[idx + 1] = mxu_part(*divmod(idx + 1, n))
            else:
                cy_s[...] = first_piece(jnp.minimum(t + 1, NT - 1))
            if idx + 1 < total:
                sv[idx + 1] = vpu_part(*divmod(idx + 1, n))
            sc = jnp.concatenate([sm.pop(idx), sv.pop(idx)], axis=0)
            if c == 0:
                o = m = None
            mc = jnp.max(sc, axis=0, keepdims=True)
            m_new = mc if m is None else jnp.maximum(m, mc)
            p = jnp.exp2(sc - m_new).astype(BF)
            oc = _dot(vt_s[g * G + i, :, c * CK:(c + 1) * CK], p)
            o = oc if o is None else o * jnp.exp2(m - m_new) + oc
            m = m_new
            if c == n - 1:
                l = o[DH:DH + 1, :]
                inv = pl.reciprocal(l, approx=True)
                inv = inv * (2.0 - l * inv)
                outs.append(o[0:DH, :] * inv)
        og = jnp.concatenate(outs, axis=0).astype(BF)
        ot_s[pl.ds(pl.multiple_of(g * GW, 16), GW), qsl] = og
        return carry

    cy_s[...] = first_piece(0)
    lax.fori_loop(0, NT, attn_body, 0)

    wo_cp.wait()
    w1_cp.wait()
    w3_cp.wait()
    w1r_cp.wait()
    w3r_cp.wait()
    w2_cp.wait()
    blocks = _p3_blocks()
    chunks = [(lo, min(FM, lo + FC)) for lo in range(0, FM, FC)]
    nfc = len(chunks)

    def out_cp(b):
        r0, sz = blocks[b]
        return pltpu.make_async_copy(out_v.at[pl.ds(r0, sz), :], out_hbm.at[pl.ds(r0, sz), :], sem_o.at[b])

    def oproj_ln(b):
        r0, sz = blocks[b]
        a = _dot_tn(ot_s[:, r0:r0 + sz], wo_v[...])
        hres = x_v[r0:r0 + sz, :].astype(F32) + a
        h_s[r0:r0 + sz, :] = hres
        hh_s[r0:r0 + sz, :] = _ln(hres).astype(BF)

    def ffn(b):
        r0, sz = blocks[b]
        hh = hh_s[r0:r0 + sz, :]

        def gu(c):
            lo, hi = chunks[c]
            gate = _dot_nt(hh, w1_v[lo:hi, :])
            up = _dot_nt(hh, w3_v[lo:hi, :])
            rem = _dot_nt(hh, wr_v[...]) if c == nfc - 1 else None
            return gate, up, rem

        cur = gu(0)
        acc = None
        for c in range(nfc):
            nxt = gu(c + 1) if c + 1 < nfc else None
            if c == 2 and b + 1 < len(blocks):
                oproj_ln(b + 1)
            gate, up, rem = cur
            lo, hi = chunks[c]
            act = (gate * jax.nn.sigmoid(gate) * up).astype(BF)
            if rem is not None:
                ur = pltpu.roll(rem, FR, 1)
                ar = (rem * jax.nn.sigmoid(rem) * ur).astype(BF)[:, 0:FR]
                act = jnp.concatenate([act, ar], axis=1)
                hi = F
            dn = _dot(act, w2_v[lo:hi, :])
            acc = dn if acc is None else acc + dn
            cur = nxt
        out_v[r0:r0 + sz, :] = (h_s[r0:r0 + sz, :] + acc).astype(BF)
        out_cp(b).start()

    oproj_ln(0)
    for b in range(len(blocks)):
        ffn(b)
    for b in range(len(blocks)):
        out_cp(b).wait()


@jax.jit
def pallas_sequential_preLN__softmax_full_mha__glu_gated_swiglu__prompt_kernel(
    A_x: jax.Array,
    A_wqkv: jax.Array,
    A_wo: jax.Array,
    B_x: jax.Array,
    B_w1: jax.Array,
    B_w3: jax.Array,
    B_w2: jax.Array,
):
    del B_x
    scratch = [
        pltpu.VMEM((S, D), BF),
        pltpu.VMEM((D, 3 * D), BF),
        pltpu.VMEM((D, D), BF),
        pltpu.VMEM((FM, D), BF),
        pltpu.VMEM((FM, D), BF),
        pltpu.VMEM((2 * FR, D), BF),
        pltpu.VMEM((F, D), BF),
        pltpu.VMEM((NG, S, 128), F32),
        pltpu.VMEM((D + 64, S), BF),
        pltpu.VMEM((H, VR, S), F32),
        pltpu.VMEM((D, S), BF),
        pltpu.VMEM((NQ, NG, GW, 8, BQ), F32),
        pltpu.VMEM((P0, BQ), F32),
        pltpu.VMEM((S, D), F32),
        pltpu.VMEM((S, D), BF),
        pltpu.VMEM((S, D), BF),
        pltpu.SemaphoreType.DMA((2,)),
        pltpu.SemaphoreType.DMA((9,)),
        pltpu.SemaphoreType.DMA((len(_p3_blocks()),)),
    ]
    anyspec = pl.BlockSpec(memory_space=pl.ANY)
    out = pl.pallas_call(
        _kernel,
        out_shape=jax.ShapeDtypeStruct((S, D), BF),
        in_specs=[anyspec] * 6,
        out_specs=anyspec,
        scratch_shapes=scratch,
        compiler_params=pltpu.CompilerParams(vmem_limit_bytes=112 * 1024 * 1024),
        name="preln_mha_swiglu_block",
    )(A_x.reshape(S, D), A_wqkv, A_wo, B_w1.T, B_w3.T, B_w2)
    return out.reshape(1, S, D)
```

```python
import numpy as np
import jax
import jax.numpy as jnp
from jax import lax
import jax.experimental.pallas as pl
import jax.experimental.pallas.tpu as pltpu

S, D, H, DH, F = 2048, 640, 32, 20, 1728
G = 4
NG = H // G
GW = G * DH
VR = 24
EPS = 1e-5
QSCALE = float(DH ** -0.5 * np.log2(np.e))
BF = jnp.bfloat16
F32 = jnp.float32
FM = (F // 128) * 128
FR = F - FM

TB1 = 256
BQ = 1024
CK = 128
VK = 8
MK = CK - VK
P0 = 72
TB3 = 256
FC = 256
NQ = S // BQ
NT = NQ * NG
NB1 = S // TB1
X0 = 2 * TB1


def _ln(xf):
    m = jnp.mean(xf, axis=-1, keepdims=True)
    d = xf - m
    v = jnp.mean(d * d, axis=-1, keepdims=True)
    return d * lax.rsqrt(v + EPS)


def _dot(a, b):
    return lax.dot_general(a, b, (((1,), (0,)), ((), ())), preferred_element_type=F32)


def _dot_nt(a, b):
    return lax.dot_general(a, b, (((1,), (1,)), ((), ())), preferred_element_type=F32)


def _dot_tn(a, b):
    return lax.dot_general(a, b, (((0,), (0,)), ((), ())), preferred_element_type=F32)


def _p3_blocks():
    blocks = [(r, TB3) for r in range(0, S - TB3, TB3)]
    blocks += [(S - TB3, TB3 // 2), (S - TB3 // 2, TB3 // 2)]
    return blocks


def _kernel(x_hbm, wqkv_hbm, wo_hbm, w1t_hbm, w3t_hbm, w2_hbm, out_hbm,
            x_v, wqkv_v, wo_v, w1_v, w3_v, wr_v, w2_v,
            k_s, qt_s, vt_s, ot_s, qr_s, cy_s, h_s, hh_s, out_v, sem_x, sem_w, sem_o):
    x0_cp = pltpu.make_async_copy(x_hbm.at[pl.ds(0, X0), :], x_v.at[pl.ds(0, X0), :], sem_x.at[0])
    x1_cp = pltpu.make_async_copy(x_hbm.at[pl.ds(X0, S - X0), :], x_v.at[pl.ds(X0, S - X0), :], sem_x.at[1])

    def wqkv_cp(j):
        return pltpu.make_async_copy(wqkv_hbm.at[:, pl.ds(j * D, D)], wqkv_v.at[:, pl.ds(j * D, D)], sem_w.at[j])

    wo_cp = pltpu.make_async_copy(wo_hbm, wo_v, sem_w.at[3])
    w1_cp = pltpu.make_async_copy(w1t_hbm.at[pl.ds(0, FM), :], w1_v, sem_w.at[4])
    w3_cp = pltpu.make_async_copy(w3t_hbm.at[pl.ds(0, FM), :], w3_v, sem_w.at[5])
    w1r_cp = pltpu.make_async_copy(w1t_hbm.at[pl.ds(FM, FR), :], wr_v.at[pl.ds(0, FR), :], sem_w.at[6])
    w3r_cp = pltpu.make_async_copy(w3t_hbm.at[pl.ds(FM, FR), :], wr_v.at[pl.ds(FR, FR), :], sem_w.at[7])
    w2_cp = pltpu.make_async_copy(w2_hbm, w2_v, sem_w.at[8])
    x0_cp.start()
    wqkv_cp(1).start()

    qt_s[D:, :] = jnp.zeros((qt_s.shape[0] - D, S), BF)

    ones_tail = (lax.broadcasted_iota(jnp.int32, (VR - DH, TB1), 0) == 0).astype(F32)
    xh = {}

    def ln1(b):
        r0 = b * TB1
        xh[b] = _ln(x_v[r0:r0 + TB1, :].astype(F32)).astype(BF)

    def qproj(b):
        r0 = b * TB1
        q = _dot(xh[b], wqkv_v[:, 0:D]) * QSCALE
        qtb = q.astype(BF).T
        qt_s[0:D, r0:r0 + TB1] = qtb
        spread_q(b, qtb)

    def spread_q(b, qtb=None):
        r0 = b * TB1
        for g in range(NG):
            if qtb is None:
                qtf = qt_s[g * GW:(g + 1) * GW, r0:r0 + TB1].astype(F32)
            else:
                qtf = qtb[g * GW:(g + 1) * GW, :].astype(F32)
            for r in range(GW):
                qr_s[r0 // BQ, g, r, :, r0 % BQ:r0 % BQ + TB1] = jnp.broadcast_to(qtf[r:r + 1, :], (8, TB1))

    def kproj(b):
        r0 = b * TB1
        k = _dot(xh[b], wqkv_v[:, D:2 * D]).astype(BF)
        kp = jnp.concatenate([k, jnp.zeros((TB1, 128), BF)], axis=1)
        for g in range(NG):
            k_s[g, r0:r0 + TB1, :] = kp[:, g * GW:g * GW + 128].astype(F32)

    def vproj(b):
        r0 = b * TB1
        vt = _dot(xh[b], wqkv_v[:, 2 * D:3 * D]).T
        for h in range(H):
            vt_s[h, :, r0:r0 + TB1] = jnp.concatenate([vt[h * DH:(h + 1) * DH, :], ones_tail], axis=0)

    x0_cp.wait()
    wqkv_cp(2).start()
    wqkv_cp(0).start()
    ln1(0)
    ln1(1)
    wqkv_cp(1).wait()
    x1_cp.start()
    kproj(0)
    kproj(1)
    wqkv_cp(2).wait()
    wqkv_cp(0).wait()
    qproj(0)
    vproj(0)
    x1_cp.wait()
    ln1(2)
    qproj(1)
    vproj(1)
    for b in range(2, NB1):
        if b + 1 < NB1:
            ln1(b + 1)
        qproj(b)
        vproj(b)
        kproj(b)

    wo_cp.start()
    w1_cp.start()
    w3_cp.start()
    w1r_cp.start()
    w3r_cp.start()
    w2_cp.start()

    n = S // CK

    def masked_q(g, ii, qsl):
        q = qt_s[pl.ds(pl.multiple_of(g * GW, 16), 128), qsl]
        qi = pltpu.bitcast(q, jnp.int32)
        r2 = lax.broadcasted_iota(jnp.int32, (64, BQ), 0)
        qi = jnp.where((r2 >= ii * (DH // 2)) & (r2 < (ii + 1) * (DH // 2)), qi, 0)
        return pltpu.bitcast(qi, BF)

    def first_piece(t):
        qb = t // NG
        g = t - qb * NG
        qsl = pl.ds(pl.multiple_of(qb * BQ, 128), BQ)
        return _dot(k_s[g, 0:P0, :], masked_q(g, 0, qsl))

    def attn_body(t, carry):
        qb = t // NG
        g = t - qb * NG
        qsl = pl.ds(pl.multiple_of(qb * BQ, 128), BQ)
        qs = {}

        def get_q(i):
            if i not in qs:
                qs[i] = masked_q(g, i, qsl)
            return qs[i]

        def mxu_part(i, c):
            q = get_q(i)
            r0 = c * CK
            if i == 0 and c == 0:
                pa = cy_s[...]
            else:
                pa = _dot(k_s[g, r0:r0 + P0, :], q)
            pb = _dot(k_s[g, r0 + P0:r0 + MK, :], q)
            return jnp.concatenate([pa, pb], axis=0)

        def vpu_part(i, c):
            r0 = c * CK + MK
            kv = k_s[g, r0:r0 + VK, :]
            accs = [None, None]
            for d in range(DH):
                r = i * DH + d
                term = kv[:, r:r + 1] * qr_s[qb, g, r]
                accs[d % 2] = term if accs[d % 2] is None else accs[d % 2] + term
            return accs[0] + accs[1]

        total = G * n
        sm = {0: mxu_part(0, 0)}
        sv = {0: vpu_part(0, 0)}
        o = m = None
        outs = []
        for idx in range(total):
            i, c = divmod(idx, n)
            if idx + 1 < total:
                sm[idx + 1] = mxu_part(*divmod(idx + 1, n))
            else:
                cy_s[...] = first_piece(jnp.minimum(t + 1, NT - 1))
            if idx + 1 < total:
                sv[idx + 1] = vpu_part(*divmod(idx + 1, n))
            sc = jnp.concatenate([sm.pop(idx), sv.pop(idx)], axis=0)
            if c == 0:
                o = m = None
            mc = jnp.max(sc, axis=0, keepdims=True)
            m_new = mc if m is None else jnp.maximum(m, mc)
            p = jnp.exp2(sc - m_new).astype(BF)
            oc = _dot(vt_s[g * G + i, :, c * CK:(c + 1) * CK], p)
            o = oc if o is None else o * jnp.exp2(m - m_new) + oc
            m = m_new
            if c == n - 1:
                l = o[DH:DH + 1, :]
                inv = pl.reciprocal(l, approx=True)
                inv = inv * (2.0 - l * inv)
                outs.append(o[0:DH, :] * inv)
        og = jnp.concatenate(outs, axis=0).astype(BF)
        ot_s[pl.ds(pl.multiple_of(g * GW, 16), GW), qsl] = og
        return carry

    cy_s[...] = first_piece(0)
    lax.fori_loop(0, NT, attn_body, 0)

    wo_cp.wait()
    w1_cp.wait()
    w3_cp.wait()
    w1r_cp.wait()
    w3r_cp.wait()
    w2_cp.wait()
    blocks = _p3_blocks()
    chunks = [(lo, min(FM, lo + FC)) for lo in range(0, FM, FC)]
    nfc = len(chunks)

    def out_cp(b):
        r0, sz = blocks[b]
        return pltpu.make_async_copy(out_v.at[pl.ds(r0, sz), :], out_hbm.at[pl.ds(r0, sz), :], sem_o.at[b])

    def oproj_ln(j):
        r0 = j * TB3
        a = _dot_tn(ot_s[:, r0:r0 + TB3], wo_v[...])
        hres = x_v[r0:r0 + TB3, :].astype(F32) + a
        h_s[r0:r0 + TB3, :] = hres
        hh_s[r0:r0 + TB3, :] = _ln(hres).astype(BF)

    def ffn(b):
        r0, sz = blocks[b]
        hh = hh_s[r0:r0 + sz, :]

        def gu(c):
            lo, hi = chunks[c]
            gate = _dot_nt(hh, w1_v[lo:hi, :])
            up = _dot_nt(hh, w3_v[lo:hi, :])
            rem = _dot_nt(hh, wr_v[...]) if c == nfc - 1 else None
            return gate, up, rem

        cur = gu(0)
        acc = None
        for c in range(nfc):
            nxt = gu(c + 1) if c + 1 < nfc else None
            if c == 2 and b + 2 < S // TB3:
                oproj_ln(b + 2)
            gate, up, rem = cur
            lo, hi = chunks[c]
            act = (gate * jax.nn.sigmoid(gate) * up).astype(BF)
            if rem is not None:
                ur = pltpu.roll(rem, FR, 1)
                ar = (rem * jax.nn.sigmoid(rem) * ur).astype(BF)[:, 0:FR]
                act = jnp.concatenate([act, ar], axis=1)
                hi = F
            dn = _dot(act, w2_v[lo:hi, :])
            acc = dn if acc is None else acc + dn
            cur = nxt
        out_v[r0:r0 + sz, :] = (h_s[r0:r0 + sz, :] + acc).astype(BF)
        out_cp(b).start()

    oproj_ln(0)
    oproj_ln(1)
    for b in range(len(blocks)):
        ffn(b)
    for b in range(len(blocks)):
        out_cp(b).wait()


@jax.jit
def pallas_sequential_preLN__softmax_full_mha__glu_gated_swiglu__prompt_kernel(
    A_x: jax.Array,
    A_wqkv: jax.Array,
    A_wo: jax.Array,
    B_x: jax.Array,
    B_w1: jax.Array,
    B_w3: jax.Array,
    B_w2: jax.Array,
):
    del B_x
    scratch = [
        pltpu.VMEM((S, D), BF),
        pltpu.VMEM((D, 3 * D), BF),
        pltpu.VMEM((D, D), BF),
        pltpu.VMEM((FM, D), BF),
        pltpu.VMEM((FM, D), BF),
        pltpu.VMEM((2 * FR, D), BF),
        pltpu.VMEM((F, D), BF),
        pltpu.VMEM((NG, S, 128), F32),
        pltpu.VMEM((D + 64, S), BF),
        pltpu.VMEM((H, VR, S), F32),
        pltpu.VMEM((D, S), BF),
        pltpu.VMEM((NQ, NG, GW, 8, BQ), F32),
        pltpu.VMEM((P0, BQ), F32),
        pltpu.VMEM((S, D), F32),
        pltpu.VMEM((S, D), BF),
        pltpu.VMEM((S, D), BF),
        pltpu.SemaphoreType.DMA((2,)),
        pltpu.SemaphoreType.DMA((9,)),
        pltpu.SemaphoreType.DMA((len(_p3_blocks()),)),
    ]
    anyspec = pl.BlockSpec(memory_space=pl.ANY)
    out = pl.pallas_call(
        _kernel,
        out_shape=jax.ShapeDtypeStruct((S, D), BF),
        in_specs=[anyspec] * 6,
        out_specs=anyspec,
        scratch_shapes=scratch,
        compiler_params=pltpu.CompilerParams(vmem_limit_bytes=112 * 1024 * 1024),
        name="preln_mha_swiglu_block",
    )(A_x.reshape(S, D), A_wqkv, A_wo, B_w1.T, B_w3.T, B_w2)
    return out.reshape(1, S, D)
```
